```python
import jax
import jax.numpy as jnp

def _softmax(x, axis=-1):
    return jax.nn.softmax(x, axis=axis)

def _gelu(x):
    return jax.nn.gelu(x, approximate=True)

def _silu(x):
    return jax.nn.silu(x)

def _sigmoid(x):
    return jax.nn.sigmoid(x)

def _layernorm(x, axis=-1, eps=1e-05):
    m = jnp.mean(x, axis=axis, keepdims=True)
    v = jnp.var(x, axis=axis, keepdims=True)
    return (x - m) / jnp.sqrt(v + eps)

def _scatter_add(tgt, idx, src, axis=0):
    return tgt.at[idx].add(src)

def _segment_sum(src, seg, n):
    return jax.ops.segment_sum(src, seg, n)

class _Rng:

    def __init__(self, key):
        self._k = key

    def _next(self):
        self._k, sub = jax.random.split(self._k)
        return sub

    def normal(self, shape):
        return jax.random.normal(self._next(), shape, dtype=jnp.bfloat16)

    def randint(self, lo, hi, shape):
        return jax.random.randint(self._next(), shape, lo, hi, dtype=jnp.int32)

    def uniform(self, shape, lo=0.0, hi=1.0):
        return jax.random.uniform(self._next(), shape, jnp.bfloat16, lo, hi)

    def permutation(self, n):
        return jax.random.permutation(self._next(), n)
kernel_name = 'adaLN_cond__sliding_local_dilated__mixer_s_mlp__prompt'

def setup_inputs():
    _rng = _Rng(jax.random.key(int.from_bytes(__import__("os").urandom(4), "little")))
    _w = lambda a: (lambda t: t.astype(jnp.bfloat16) if jnp.issubdtype(t.dtype, jnp.floating) else t)(jnp.asarray(a))

    def _A_setup():
        B, S, D = (1, 2048, 1024)
        return {'x': _w((lambda *s: _rng.normal(s) * 0.05)(B, S, D)), 'wqkv': _w((lambda *s: _rng.normal(s) * 0.05)(D, 3 * D)), 'wo': _w((lambda *s: _rng.normal(s) * 0.05)(D, D))}
    _A_in = _A_setup()

    def _B_setup():
        B, S, D, F = (1, 2048, 1024, 3584)
        return {'x': _w((lambda *s: _rng.normal(s) * 0.05)(B, S, D)), 'w1': _w((lambda *s: _rng.normal(s) * 0.05)(D, D) * D ** (-0.5)), 'w2': _w((lambda *s: _rng.normal(s) * 0.05)(D, D) * D ** (-0.5)), 'w3': _w((lambda *s: _rng.normal(s) * 0.05)(D, F) * D ** (-0.5)), 'w4': _w((lambda *s: _rng.normal(s) * 0.05)(F, D) * F ** (-0.5))}
    _B_in = _B_setup()
    return {'A_x': _A_in['x'], 'A_wqkv': _A_in['wqkv'], 'A_wo': _A_in['wo'], 'B_x': _B_in['x'], 'B_w1': _B_in['w1'], 'B_w2': _B_in['w2'], 'B_w3': _B_in['w3'], 'B_w4': _B_in['w4'], 'c': _w((lambda *s: _rng.normal(s) * 0.05)(1, 1024)), 'w_mod': _w((lambda *s: _rng.normal(s) * 0.05)(1024, 6 * 1024) * 1024 ** (-0.5))}

def reference(A_x, A_wqkv, A_wo, B_x, B_w1, B_w2, B_w3, B_w4, c, w_mod):

    def _A_ref(x, wqkv, wo):
        B, S, D = x.shape
        H = 32
        Dh = D // H
        W, dil = (8, 2)
        qkv = (lambda x, *d: x.transpose(*d))((x @ wqkv).reshape(B, S, 3, H, Dh), 2, 0, 3, 1, 4)
        q, k, v = (qkv[0], qkv[1], qkv[2])
        scale = Dh ** (-0.5)
        pos = jnp.arange(S)
        off = jnp.arange(W) * dil
        idx = pos[:, None] - off[None, :]
        mask = idx >= 0
        idx_c = jnp.where(mask, idx, 0).reshape(-1)
        kg = k[:, :, idx_c, :].reshape(B, H, S, W, Dh)
        vg = v[:, :, idx_c, :].reshape(B, H, S, W, Dh)
        logits = jnp.einsum('bhsd,bhswd->bhsw', q, kg) * scale
        logits = jnp.where(mask[None, None, :, :], logits, -1000000000.0)
        attn = _softmax(logits, axis=-1)
        o = jnp.einsum('bhsw,bhswd->bhsd', attn, vg)
        return (lambda x, *d: x.transpose(*d))(o, 0, 2, 1, 3).reshape(B, S, D) @ wo

    def _B_ref(x, w1, w2, w3, w4):
        B, S, D = x.shape
        h = _gelu(_layernorm(x, axis=-1) @ w1)
        c = D // 4
        g0 = jnp.pad(h[:, :, 0 * c:1 * c], ((0, 0), (1, 0), (0, 0)))[:, :S, :]
        g1 = jnp.pad(h[:, :, 1 * c:2 * c], ((0, 0), (0, 1), (0, 0)))[:, 1:, :]
        g2 = jnp.pad(h[:, :, 2 * c:3 * c], ((0, 0), (2, 0), (0, 0)))[:, :S, :]
        g3 = jnp.pad(h[:, :, 3 * c:], ((0, 0), (0, 2), (0, 0)))[:, 2:, :]
        hs = jnp.concatenate([g0, g1, g2, g3], axis=-1) @ w2
        x1 = x + hs
        h2 = _gelu(_layernorm(x1, axis=-1) @ w3) @ w4
        return x1 + h2
    x = A_x
    mod = (_silu(c) @ w_mod).reshape(c.shape[0], 6, 1, -1)
    sa, ca, ga, sb, cb, gb = (mod[:, 0].copy(), mod[:, 1].copy(), mod[:, 2].copy(), mod[:, 3].copy(), mod[:, 4].copy(), mod[:, 5].copy())
    h = _layernorm(x, axis=-1) * (1 + ca) + sa
    x = x + ga * _A_ref(h, A_wqkv, A_wo)
    h = _layernorm(x, axis=-1) * (1 + cb) + sb
    x = x + gb * _B_ref(h, B_w1, B_w2, B_w3, B_w4)
    return x
```

```python
import jax
import jax.numpy as jnp
from jax import lax
import jax.experimental.pallas as pl
import jax.experimental.pallas.tpu as pltpu

S, D, F = 2048, 1024, 3584
H, DH, W, DIL = 32, 32, 8, 2
T = 256
NB = S // T
NC = D // 128
PAD = 16
FC = 512
F32, BF16 = jnp.float32, jnp.bfloat16


def _ln(x):
    m = jnp.mean(x, axis=-1, keepdims=True)
    d = x - m
    v = jnp.mean(d * d, axis=-1, keepdims=True)
    return d * lax.rsqrt(v + 1e-5)


def _gelu(x):
    u = 0.7978845608028654 * (x + 0.044715 * (x * x * x))
    return 0.5 * x * (1.0 + jnp.tanh(u))


def _dot(a, b):
    return jnp.dot(a, b, preferred_element_type=F32)


def _body(x_ref, c_ref, wqkv_h, wo_h, w1_h, w2_h, w3_h, w4_h, wmod_h, o_ref,
          wqkv, wo, w1, w2, w3, w4, wmod, mod, kbuf, vbuf, obuf, xres, hb, hbuf, sems):
    ph = pl.program_id(0)
    i = pl.program_id(1)

    def cp(n):
        src, dst = [
            (wmod_h.at[:, 0:2 * D], wmod.at[:, 0:2 * D]),
            (wqkv_h, wqkv),
            (wo_h, wo),
            (wmod_h.at[:, 2 * D:], wmod.at[:, 2 * D:]),
            (w1_h, w1), (w2_h, w2), (w3_h, w3), (w4_h, w4)][n]
        return pltpu.make_async_copy(src, dst, sems.at[n])

    def silu_c():
        c = c_ref[...].astype(F32)
        return jnp.broadcast_to(c * jax.nn.sigmoid(c), (8, D)).astype(BF16)

    @pl.when((ph == 0) & (i == 0))
    def _():
        cp(0).start()
        cp(1).start()
        kbuf[:, 0:PAD, :] = jnp.zeros((NC, PAD, 128), F32)
        vbuf[:, 0:PAD, :] = jnp.zeros((NC, PAD, 128), F32)
        hbuf[:, 0:8, :] = jnp.zeros((NC, 8, 128), F32)
        hbuf[:, S + 8:S + 16, :] = jnp.zeros((NC, 8, 128), F32)
        cp(0).wait()
        mod[:, 0:2 * D] = _dot(silu_c(), wmod[:, 0:2 * D])
        cp(1).wait()
        for n in range(2, 8):
            cp(n).start()

    @pl.when((ph == 1) & (i == 0))
    def _():
        cp(2).wait()
        cp(3).wait()
        cp(4).wait()
        mod[:, 2 * D:] = _dot(silu_c(), wmod[:, 2 * D:])

    @pl.when((ph == 2) & (i == 0))
    def _():
        cp(5).wait()
        cp(6).wait()
        cp(7).wait()

    def m(k):
        return mod[0:1, k * D:(k + 1) * D]

    rows = pl.ds(pl.multiple_of(i * T, T), T)

    @pl.when(ph == 0)
    def _():
        x = x_ref[...].astype(F32)
        h = (_ln(x) * (1.0 + m(1)) + m(0)).astype(BF16)
        k = _dot(h, wqkv[:, D:2 * D])
        v = _dot(h, wqkv[:, 2 * D:])
        for c in range(NC):
            kbuf[c, PAD:, :] = k[:, c * 128:(c + 1) * 128]
            vbuf[c, PAD:, :] = v[:, c * 128:(c + 1) * 128]
        q = _dot(h, wqkv[:, 0:D]) * (DH ** -0.5)
        r0 = lax.broadcasted_iota(jnp.int32, (128, 128), 0) // DH
        r1 = lax.broadcasted_iota(jnp.int32, (128, 128), 1) // DH
        e = (r0 == r1).astype(BF16)
        pos = lax.broadcasted_iota(jnp.int32, (T, 128), 0) + i * T
        for c in range(NC):
            qc = q[:, c * 128:(c + 1) * 128]
            lg = []
            for w in range(W):
                p = (qc * kbuf[c, pl.ds(PAD - DIL * w, T), :]).astype(BF16)
                l = _dot(p, e)
                if w:
                    l = jnp.where(pos >= DIL * w, l, -1e9)
                lg.append(l)
            mx = lg[0]
            for w in range(1, W):
                mx = jnp.maximum(mx, lg[w])
            den = None
            acc = None
            for w in range(W):
                ew = jnp.exp(lg[w] - mx)
                t = ew * vbuf[c, pl.ds(PAD - DIL * w, T), :]
                den = ew if w == 0 else den + ew
                acc = t if w == 0 else acc + t
            obuf[rows, c * 128:(c + 1) * 128] = (acc * pl.reciprocal(den)).astype(BF16)
        kbuf[:, 0:PAD, :] = kbuf[:, T:T + PAD, :]
        vbuf[:, 0:PAD, :] = vbuf[:, T:T + PAD, :]

    @pl.when(ph == 1)
    def _():
        x = x_ref[...].astype(F32) + m(2) * _dot(obuf[rows, :], wo[...])
        xres[rows, :] = x
        g = _ln(x) * (1.0 + m(4)) + m(3)
        hb[rows, :] = g
        h = _gelu(_dot(_ln(g).astype(BF16), w1[...]))
        for c in range(NC):
            hbuf[c, pl.ds(pl.multiple_of(i * T, T) + 8, T), :] = h[:, c * 128:(c + 1) * 128]

    @pl.when(ph == 2)
    def _():
        shifts = (-1, 1, -2, 2)
        parts = []
        for c in range(NC):
            win = hbuf[c, pl.ds(pl.multiple_of(i * T, T), T + 16), :]
            s = 8 + shifts[c // 2]
            parts.append(win[s:s + T].astype(BF16))
        x1 = hb[rows, :] + _dot(jnp.concatenate(parts, axis=1), w2[...])
        n = _ln(x1).astype(BF16)
        acc = x1
        for f in range(F // FC):
            u = _gelu(_dot(n, w3[:, f * FC:(f + 1) * FC])).astype(BF16)
            acc = acc + _dot(u, w4[f * FC:(f + 1) * FC, :])
        o_ref[...] = (xres[rows, :] + m(5) * acc).astype(o_ref.dtype)


@jax.jit
def pallas_adaLN_cond__sliding_local_dilated__mixer_s_mlp__prompt_kernel(
        A_x, A_wqkv, A_wo, B_x, B_w1, B_w2, B_w3, B_w4, c, w_mod):
    del B_x
    anyspec = pl.BlockSpec(memory_space=pl.ANY)
    out = pl.pallas_call(
        _body,
        grid=(3, NB),
        in_specs=[pl.BlockSpec((T, D), lambda p, i: (jnp.where(p < 2, i, NB - 1), 0)),
                  pl.BlockSpec((1, D), lambda p, i: (0, 0))] + [anyspec] * 7,
        out_specs=pl.BlockSpec((T, D), lambda p, i: (jnp.where(p == 2, i, 0), 0)),
        out_shape=jax.ShapeDtypeStruct((S, D), A_x.dtype),
        scratch_shapes=[
            pltpu.VMEM((D, 3 * D), BF16), pltpu.VMEM((D, D), BF16),
            pltpu.VMEM((D, D), BF16), pltpu.VMEM((D, D), BF16),
            pltpu.VMEM((D, F), BF16), pltpu.VMEM((F, D), BF16),
            pltpu.VMEM((D, 6 * D), BF16), pltpu.VMEM((8, 6 * D), F32),
            pltpu.VMEM((NC, T + PAD, 128), F32), pltpu.VMEM((NC, T + PAD, 128), F32),
            pltpu.VMEM((S, D), BF16), pltpu.VMEM((S, D), F32), pltpu.VMEM((S, D), F32),
            pltpu.VMEM((NC, S + 16, 128), F32),
            pltpu.SemaphoreType.DMA((8,)),
        ],
        compiler_params=pltpu.CompilerParams(
            dimension_semantics=("arbitrary", "arbitrary"),
            vmem_limit_bytes=110 * 1024 * 1024),
    )(A_x.reshape(S, D), c, A_wqkv, A_wo, B_w1, B_w2, B_w3, B_w4, w_mod)
    return out.reshape(1, S, D)
```

```python
import jax
import jax.numpy as jnp
from jax import lax
import jax.experimental.pallas as pl
import jax.experimental.pallas.tpu as pltpu

S, D, F = 2048, 1024, 3584
H, DH, W, DIL = 32, 32, 8, 2
T = 256
NB = S // T
NC = D // 128
HG = 8
PAD = 128
FC = 512
F32, BF16 = jnp.float32, jnp.bfloat16


def _ln(x):
    m = jnp.mean(x, axis=-1, keepdims=True)
    d = x - m
    v = jnp.mean(d * d, axis=-1, keepdims=True)
    return d * lax.rsqrt(v + 1e-5)


def _gelu(x):
    u = 0.7978845608028654 * (x + 0.044715 * (x * x * x))
    return 0.5 * x * (1.0 + jnp.tanh(u))


def _dot(a, b):
    return jnp.dot(a, b, preferred_element_type=F32)


def _body(x_ref, c_ref, wqkv_h, wo_h, w1_h, w2_h, w3_h, w4_h, wmod_h, o_ref,
          wqkv, wo, w1, w2, w3, w4, wmod, mod, kbuf, vbuf, qbuf, kn, vn, qn, obuf, xres, hb, hbuf, sems):
    ph = pl.program_id(0)
    i = pl.program_id(1)

    def cp(n):
        src, dst = [
            (wmod_h.at[:, 0:2 * D], wmod.at[:, 0:2 * D]),
            (wqkv_h, wqkv),
            (wo_h, wo),
            (wmod_h.at[:, 2 * D:], wmod.at[:, 2 * D:]),
            (w1_h, w1), (w2_h, w2), (w3_h, w3), (w4_h, w4)][n]
        return pltpu.make_async_copy(src, dst, sems.at[n])

    def silu_c():
        c = c_ref[...].astype(F32)
        return jnp.broadcast_to(c * jax.nn.sigmoid(c), (8, D)).astype(BF16)

    @pl.when((ph == 0) & (i == 0))
    def _():
        cp(0).start()
        cp(1).start()
        kbuf[...] = jnp.zeros((D, T + PAD), BF16)
        vbuf[...] = jnp.zeros((D, T + PAD), BF16)
        qbuf[...] = jnp.zeros((D, T), BF16)
        hbuf[:, 0:8, :] = jnp.zeros((NC, 8, 128), F32)
        hbuf[:, S + 8:S + 16, :] = jnp.zeros((NC, 8, 128), F32)
        cp(0).wait()
        mod[:, 0:2 * D] = _dot(silu_c(), wmod[:, 0:2 * D])
        cp(1).wait()
        for n in range(2, 8):
            cp(n).start()

    @pl.when((ph == 1) & (i == 0))
    def _():
        cp(2).wait()
        cp(3).wait()
        cp(4).wait()
        sc = silu_c()

        @pl.loop(2, 6)
        def _(k):
            cols = pl.ds(pl.multiple_of(k * D, D), D)
            mod[:, cols] = _dot(sc, wmod[:, cols])

    @pl.when((ph == 2) & (i == 0))
    def _():
        cp(5).wait()
        cp(6).wait()
        cp(7).wait()

    def m(k):
        return mod[0:1, k * D:(k + 1) * D]

    rows = pl.ds(pl.multiple_of(i * T, T), T)

    def qkv():
        x = x_ref[...].astype(F32)
        h = (_ln(x) * (1.0 + m(1)) + m(0)).astype(BF16)
        kn[...] = _dot(h, wqkv[:, D:2 * D]).astype(BF16).T
        vn[...] = _dot(h, wqkv[:, 2 * D:]).astype(BF16).T
        qn[...] = _dot(h, wqkv[:, 0:D]).astype(BF16).T

    def attn(j):
        G = HG * DH
        pos = lax.broadcasted_iota(jnp.int32, (HG, T), 1) + j * T
        outs = []
        for g in range(D // G):
            fs = slice(g * G, (g + 1) * G)
            qg = qbuf[fs, :].astype(F32) * (DH ** -0.5)
            kg = kbuf[fs, :]
            vg = vbuf[fs, :]
            lg = []
            for w in range(W):
                o = PAD - DIL * w
                l = (qg * kg[:, o:o + T].astype(F32)).reshape(HG, DH, T).sum(axis=1)
                if w:
                    l = jnp.where(pos >= DIL * w, l, -1e9)
                lg.append(l)
            mx = lg[0]
            for w in range(1, W):
                mx = jnp.maximum(mx, lg[w])
            ex = [jnp.exp(l - mx) for l in lg]
            den = ex[0]
            for w in range(1, W):
                den = den + ex[w]
            r = pl.reciprocal(den)
            acc = None
            for w in range(W):
                o = PAD - DIL * w
                t = (ex[w] * r)[:, None, :] * vg[:, o:o + T].astype(F32).reshape(HG, DH, T)
                acc = t if w == 0 else acc + t
            outs.append(acc.reshape(G, T).astype(BF16))
        obuf[pl.ds(pl.multiple_of(j * T, T), T), :] = jnp.concatenate(outs, axis=0).T
        kbuf[:, 0:PAD] = kbuf[:, T:T + PAD]
        vbuf[:, 0:PAD] = vbuf[:, T:T + PAD]

    @pl.when(ph == 0)
    def _():
        qkv()
        attn(jnp.maximum(i - 1, 0))
        kbuf[:, PAD:] = kn[...]
        vbuf[:, PAD:] = vn[...]
        qbuf[...] = qn[...]

    @pl.when((ph == 1) & (i == 0))
    def _():
        attn(NB - 1)

    @pl.when(ph == 1)
    def _():
        x = x_ref[...].astype(F32) + m(2) * _dot(obuf[rows, :], wo[...])
        xres[rows, :] = x
        g = _ln(x) * (1.0 + m(4)) + m(3)
        hb[rows, :] = g
        h = _gelu(_dot(_ln(g).astype(BF16), w1[...]))
        for c in range(NC):
            hbuf[c, pl.ds(pl.multiple_of(i * T, T) + 8, T), :] = h[:, c * 128:(c + 1) * 128]

    @pl.when(ph == 2)
    def _():
        shifts = (-1, 1, -2, 2)
        parts = []
        for c in range(NC):
            win = hbuf[c, pl.ds(pl.multiple_of(i * T, T), T + 16), :]
            s = 8 + shifts[c // 2]
            parts.append(win[s:s + T].astype(BF16))
        x1 = hb[rows, :] + _dot(jnp.concatenate(parts, axis=1), w2[...])
        n = _ln(x1).astype(BF16)
        acc = x1
        for f in range(F // FC):
            u = _gelu(_dot(n, w3[:, f * FC:(f + 1) * FC])).astype(BF16)
            acc = acc + _dot(u, w4[f * FC:(f + 1) * FC, :])
        o_ref[...] = (xres[rows, :] + m(5) * acc).astype(o_ref.dtype)


@jax.jit
def pallas_adaLN_cond__sliding_local_dilated__mixer_s_mlp__prompt_kernel(
        A_x, A_wqkv, A_wo, B_x, B_w1, B_w2, B_w3, B_w4, c, w_mod):
    del B_x
    anyspec = pl.BlockSpec(memory_space=pl.ANY)
    out = pl.pallas_call(
        _body,
        grid=(3, NB),
        in_specs=[pl.BlockSpec((T, D), lambda p, i: (jnp.where(p < 2, i, NB - 1), 0)),
                  pl.BlockSpec((1, D), lambda p, i: (0, 0))] + [anyspec] * 7,
        out_specs=pl.BlockSpec((T, D), lambda p, i: (jnp.where(p == 2, i, 0), 0)),
        out_shape=jax.ShapeDtypeStruct((S, D), A_x.dtype),
        scratch_shapes=[
            pltpu.VMEM((D, 3 * D), BF16), pltpu.VMEM((D, D), BF16),
            pltpu.VMEM((D, D), BF16), pltpu.VMEM((D, D), BF16),
            pltpu.VMEM((D, F), BF16), pltpu.VMEM((F, D), BF16),
            pltpu.VMEM((D, 6 * D), BF16), pltpu.VMEM((8, 6 * D), F32),
            pltpu.VMEM((D, T + PAD), BF16), pltpu.VMEM((D, T + PAD), BF16),
            *[pltpu.VMEM((D, T), BF16)] * 4,
            pltpu.VMEM((S, D), BF16), pltpu.VMEM((S, D), F32), pltpu.VMEM((S, D), F32),
            pltpu.VMEM((NC, S + 16, 128), F32),
            pltpu.SemaphoreType.DMA((8,)),
        ],
        compiler_params=pltpu.CompilerParams(
            dimension_semantics=("arbitrary", "arbitrary"),
            vmem_limit_bytes=110 * 1024 * 1024),
    )(A_x.reshape(S, D), c, A_wqkv, A_wo, B_w1, B_w2, B_w3, B_w4, w_mod)
    return out.reshape(1, S, D)
```

```python
import jax
import jax.numpy as jnp
from jax import lax
import jax.experimental.pallas as pl
import jax.experimental.pallas.tpu as pltpu

S, D, F = 2048, 1024, 3584
H, DH, W, DIL = 32, 32, 8, 2
T = 256
NB = S // T
NC = D // 128
HG = 8
PAD = 128
FC = 512
F32, BF16 = jnp.float32, jnp.bfloat16


def _ln(x):
    m = jnp.mean(x, axis=-1, keepdims=True)
    d = x - m
    v = jnp.mean(d * d, axis=-1, keepdims=True)
    return d * lax.rsqrt(v + 1e-5)


def _gelu(x):
    u = 0.7978845608028654 * (x + 0.044715 * (x * x * x))
    return 0.5 * x * (1.0 + jnp.tanh(u))


def _dot(a, b):
    return jnp.dot(a, b, preferred_element_type=F32)


def _body(x_ref, c_ref, wqkv_h, wo_h, w1_h, w2_h, w3_h, w4_h, wmod_h, o_ref,
          wqkv, wo, w1, w2, w3, w4, wmod, mod, kbuf, vbuf, qbuf, kn, vn, qn, obuf, xres, hb, hbuf, sems):
    ph = pl.program_id(0)
    i = pl.program_id(1)

    def cp(n):
        src, dst = [
            (wmod_h.at[:, 0:2 * D], wmod.at[:, 0:2 * D]),
            (wqkv_h, wqkv),
            (wo_h, wo),
            (wmod_h.at[:, 2 * D:], wmod.at[:, 2 * D:]),
            (w1_h, w1), (w2_h, w2), (w3_h, w3), (w4_h, w4)][n]
        return pltpu.make_async_copy(src, dst, sems.at[n])

    def silu_c():
        c = c_ref[...].astype(F32)
        return jnp.broadcast_to(c * jax.nn.sigmoid(c), (8, D)).astype(BF16)

    @pl.when((ph == 0) & (i == 0))
    def _():
        cp(0).start()
        cp(1).start()
        kbuf[...] = jnp.zeros((D, T + PAD), BF16)
        vbuf[...] = jnp.zeros((D, T + PAD), BF16)
        qbuf[...] = jnp.zeros((D, T), BF16)
        hbuf[:, 0:8, :] = jnp.zeros((NC, 8, 128), F32)
        hbuf[:, S + 8:S + 16, :] = jnp.zeros((NC, 8, 128), F32)
        cp(0).wait()
        mod[:, 0:2 * D] = _dot(silu_c(), wmod[:, 0:2 * D])
        cp(1).wait()

    for st, ns in ((0, (2, 4)), (1, (3,)), (2, (5,)), (3, (6,)), (4, (7,))):
        @pl.when((ph == 0) & (i == st))
        def _():
            for n in ns:
                cp(n).start()

    @pl.when((ph == 1) & (i == 0))
    def _():
        cp(2).wait()
        cp(3).wait()
        cp(4).wait()
        sc = silu_c()

        @pl.loop(2, 6)
        def _(k):
            cols = pl.ds(pl.multiple_of(k * D, D), D)
            mod[:, cols] = _dot(sc, wmod[:, cols])

    @pl.when((ph == 2) & (i == 0))
    def _():
        cp(5).wait()
        cp(6).wait()
        cp(7).wait()

    def m(k):
        return mod[0:1, k * D:(k + 1) * D]

    rows = pl.ds(pl.multiple_of(i * T, T), T)

    def qkv():
        x = x_ref[...].astype(F32)
        h = (_ln(x) * (1.0 + m(1)) + m(0)).astype(BF16)
        kn[...] = _dot(h, wqkv[:, D:2 * D]).astype(BF16).T
        vn[...] = _dot(h, wqkv[:, 2 * D:]).astype(BF16).T
        qn[...] = _dot(h, wqkv[:, 0:D]).astype(BF16).T

    def attn(j):
        G = HG * DH
        pos = lax.broadcasted_iota(jnp.int32, (HG, T), 1) + j * T
        outs = []
        for g in range(D // G):
            fs = slice(g * G, (g + 1) * G)
            qg = qbuf[fs, :].astype(F32) * (DH ** -0.5)
            kg = kbuf[fs, :]
            vg = vbuf[fs, :]
            lg = []
            for w in range(W):
                o = PAD - DIL * w
                l = (qg * kg[:, o:o + T].astype(F32)).reshape(HG, DH, T).sum(axis=1)
                if w:
                    l = jnp.where(pos >= DIL * w, l, -1e9)
                lg.append(l)
            mx = lg[0]
            for w in range(1, W):
                mx = jnp.maximum(mx, lg[w])
            ex = [jnp.exp(l - mx) for l in lg]
            den = ex[0]
            for w in range(1, W):
                den = den + ex[w]
            r = pl.reciprocal(den)
            acc = None
            for w in range(W):
                o = PAD - DIL * w
                t = (ex[w] * r)[:, None, :] * vg[:, o:o + T].astype(F32).reshape(HG, DH, T)
                acc = t if w == 0 else acc + t
            outs.append(acc.reshape(G, T).astype(BF16))
        obuf[pl.ds(pl.multiple_of(j * T, T), T), :] = jnp.concatenate(outs, axis=0).T
        kbuf[:, 0:PAD] = kbuf[:, T:T + PAD]
        vbuf[:, 0:PAD] = vbuf[:, T:T + PAD]

    @pl.when(ph == 0)
    def _():
        qkv()
        attn(jnp.maximum(i - 1, 0))
        kbuf[:, PAD:] = kn[...]
        vbuf[:, PAD:] = vn[...]
        qbuf[...] = qn[...]

    @pl.when((ph == 1) & (i == 0))
    def _():
        attn(NB - 1)

    @pl.when(ph == 1)
    def _():
        x = x_ref[...].astype(F32) + m(2) * _dot(obuf[rows, :], wo[...])
        xres[rows, :] = x
        g = _ln(x) * (1.0 + m(4)) + m(3)
        hb[rows, :] = g
        h = _gelu(_dot(_ln(g).astype(BF16), w1[...]))
        for c in range(NC):
            hbuf[c, pl.ds(pl.multiple_of(i * T, T) + 8, T), :] = h[:, c * 128:(c + 1) * 128]

    @pl.when(ph == 2)
    def _():
        shifts = (-1, 1, -2, 2)
        parts = []
        for c in range(NC):
            win = hbuf[c, pl.ds(pl.multiple_of(i * T, T), T + 16), :]
            s = 8 + shifts[c // 2]
            parts.append(win[s:s + T].astype(BF16))
        x1 = hb[rows, :] + _dot(jnp.concatenate(parts, axis=1), w2[...])
        n = _ln(x1).astype(BF16)
        acc = x1
        for f in range(F // FC):
            u = _gelu(_dot(n, w3[:, f * FC:(f + 1) * FC])).astype(BF16)
            acc = acc + _dot(u, w4[f * FC:(f + 1) * FC, :])
        o_ref[...] = (xres[rows, :] + m(5) * acc).astype(o_ref.dtype)


@jax.jit
def pallas_adaLN_cond__sliding_local_dilated__mixer_s_mlp__prompt_kernel(
        A_x, A_wqkv, A_wo, B_x, B_w1, B_w2, B_w3, B_w4, c, w_mod):
    del B_x
    anyspec = pl.BlockSpec(memory_space=pl.ANY)
    out = pl.pallas_call(
        _body,
        grid=(3, NB),
        in_specs=[pl.BlockSpec((T, D), lambda p, i: (jnp.where(p < 2, i, NB - 1), 0)),
                  pl.BlockSpec((1, D), lambda p, i: (0, 0))] + [anyspec] * 7,
        out_specs=pl.BlockSpec((T, D), lambda p, i: (jnp.where(p == 2, i, 0), 0)),
        out_shape=jax.ShapeDtypeStruct((S, D), A_x.dtype),
        scratch_shapes=[
            pltpu.VMEM((D, 3 * D), BF16), pltpu.VMEM((D, D), BF16),
            pltpu.VMEM((D, D), BF16), pltpu.VMEM((D, D), BF16),
            pltpu.VMEM((D, F), BF16), pltpu.VMEM((F, D), BF16),
            pltpu.VMEM((D, 6 * D), BF16), pltpu.VMEM((8, 6 * D), F32),
            pltpu.VMEM((D, T + PAD), BF16), pltpu.VMEM((D, T + PAD), BF16),
            *[pltpu.VMEM((D, T), BF16)] * 4,
            pltpu.VMEM((S, D), BF16), pltpu.VMEM((S, D), F32), pltpu.VMEM((S, D), F32),
            pltpu.VMEM((NC, S + 16, 128), F32),
            pltpu.SemaphoreType.DMA((8,)),
        ],
        compiler_params=pltpu.CompilerParams(
            dimension_semantics=("arbitrary", "arbitrary"),
            vmem_limit_bytes=110 * 1024 * 1024),
    )(A_x.reshape(S, D), c, A_wqkv, A_wo, B_w1, B_w2, B_w3, B_w4, w_mod)
    return out.reshape(1, S, D)
```
